```python
import os as _os
_os.environ.setdefault("JAX_PLATFORMS", "cpu")
import jax
import jax.numpy as jnp

def _softmax(x, axis=-1):
    return jax.nn.softmax(x, axis=axis)
def _gelu(x):
    return jax.nn.gelu(x, approximate=True)
def _silu(x):
    return jax.nn.silu(x)
def _sigmoid(x):
    return jax.nn.sigmoid(x)
def _layernorm(x, axis=-1, eps=1e-5):
    m = jnp.mean(x, axis=axis, keepdims=True)
    v = jnp.var(x, axis=axis, keepdims=True)
    return (x - m) / jnp.sqrt(v + eps)
def _scatter_add(tgt, idx, src, axis=0):
    return tgt.at[idx].add(src)
def _segment_sum(src, seg, n):
    return jax.ops.segment_sum(src, seg, n)
class _Rng:
    def __init__(self, key):
        self._k = key
    def _next(self):
        self._k, sub = jax.random.split(self._k)
        return sub
    def normal(self, shape):
        return jax.random.normal(self._next(), shape, dtype=jnp.bfloat16)
    def randint(self, lo, hi, shape):
        return jax.random.randint(self._next(), shape, lo, hi, dtype=jnp.int32)
    def uniform(self, shape, lo=0.0, hi=1.0):
        return jax.random.uniform(self._next(), shape, jnp.bfloat16, lo, hi)
    def permutation(self, n):
        return jax.random.permutation(self._next(), n)


kernel_name = 'sequential_preLN__mha_block__moe_arch_mod__prompt'

def setup_inputs():
    _rng = _Rng(jax.random.key(int.from_bytes(__import__("os").urandom(4), "little")))
    _w = (lambda a: (lambda t: t.astype(jnp.bfloat16) if jnp.issubdtype(t.dtype, jnp.floating) else t)(jnp.asarray(a)))
    def _A_setup():
        B, S, D, H = 1, 2048, 640, 32
        return {
            "x": _w((lambda *s: _rng.normal(s) * 0.05)(B, S, D)),
            "wqkv": _w((lambda *s: _rng.normal(s) * 0.05)(D, 3 * D)),
            "wo": _w((lambda *s: _rng.normal(s) * 0.05)(D, D)),
        }
    _A_in = _A_setup()

    def _B_setup():
        B, S, D, F, C = 1, 2048, 640, 1536, 1
        return {
            "x": _w((lambda *s: _rng.normal(s) * 0.05)(B, S, D)),
            "w_r": _w((lambda *s: _rng.normal(s) * 0.05)(D)),
            "w_gate": _w((lambda *s: _rng.normal(s) * 0.05)(D, F)),
            "w_up": _w((lambda *s: _rng.normal(s) * 0.05)(D, F)),
            "w_down": _w((lambda *s: _rng.normal(s) * 0.05)(F, D)),
        }
    _B_in = _B_setup()

    return {
        "A_x": _A_in["x"],
        "A_wqkv": _A_in["wqkv"],
        "A_wo": _A_in["wo"],
        "B_x": _B_in["x"],
        "B_w_r": _B_in["w_r"],
        "B_w_gate": _B_in["w_gate"],
        "B_w_up": _B_in["w_up"],
        "B_w_down": _B_in["w_down"],
    }

def reference(A_x, A_wqkv, A_wo, B_x, B_w_r, B_w_gate, B_w_up, B_w_down):
    def _A_ref(x, wqkv, wo):
        B, S, D = x.shape
        H = 32
        Dh = D // H
        qkv = (lambda x, *d: x.transpose(*d))((x @ wqkv).reshape(B, S, 3, H, Dh), 2, 0, 3, 1, 4)
        q, k, v = qkv[0], qkv[1], qkv[2]
        scores = jnp.einsum("bhqd,bhkd->bhqk", q, k) * (Dh ** -0.5)
        p = _softmax(scores, axis=-1)
        o = jnp.einsum("bhqk,bhkd->bhqd", p, v)
        return (lambda x, *d: x.transpose(*d))(o, 0, 2, 1, 3).reshape(B, S, D) @ wo

    def _B_ref(x, w_r, w_gate, w_up, w_down):
        B, S, D = x.shape
        C = 1
        r = x @ w_r
        idx = jnp.argsort(-r, axis=-1)[:, :C]
        idx_e = jnp.repeat(idx.reshape(B, C, 1), D, axis=2)
        x_sel = jnp.take_along_axis(x, idx_e, axis=1)
        g = _silu(x_sel @ w_gate)
        u = x_sel @ w_up
        y = (g * u) @ w_down
        r_sel = _sigmoid(jnp.take_along_axis(r, idx, axis=1))
        y = y * r_sel.reshape(B, C, 1)
        b_off = (jnp.arange(B) * S).reshape(B, 1)
        flat_idx = (idx + b_off).reshape(B * C)
        zero = (x * 0.0).reshape(B * S, D)
        upd = _scatter_add(zero, flat_idx, y.reshape(B * C, D), axis=0)
        return x + upd.reshape(B, S, D)

    x = A_x
    h = x + _A_ref(_layernorm(x, axis=-1), A_wqkv, A_wo)
    h2 = h + _B_ref(_layernorm(h, axis=-1), B_w_r, B_w_gate, B_w_up, B_w_down)
    return h2
```

```python
import jax
import jax.numpy as jnp
import jax.experimental.pallas as pl
import jax.experimental.pallas.tpu as pltpu

S, D, H, DH, F = 2048, 640, 32, 20, 1536
HP = 32
NW = 8
LOG2E = 1.4426950408889634

def make_kernel(MQ):
    NQB = S // MQ
    def kernel(x_ref, wqT_ref, wk_ref, wvT_ref, wo_ref, wr_ref, wg_ref, wu_ref, wd_ref, o_ref,
               k_sc, qT_sc, vT_sc, oT_sc):
        x = x_ref[...].astype(jnp.float32)
        mu = jnp.mean(x, axis=-1, keepdims=True)
        xc = x - mu
        var = jnp.mean(xc * xc, axis=-1, keepdims=True)
        xn = (xc * jax.lax.rsqrt(var + 1e-5)).astype(jnp.bfloat16)
        scale = (DH ** -0.5) * LOG2E
        rowi = jax.lax.broadcasted_iota(jnp.int32, (128, S), 0)
        onesrow = (rowi % HP) == DH
        for w in range(NW):
            k_sc[w] = jnp.dot(xn, wk_ref[:, w * 128:(w + 1) * 128],
                              preferred_element_type=jnp.float32).astype(jnp.bfloat16)
            qT = jax.lax.dot_general(wqT_ref[w * 128:(w + 1) * 128, :], xn, (((1,), (1,)), ((), ())),
                                     preferred_element_type=jnp.float32)
            qT_sc[w] = (qT * scale).astype(jnp.bfloat16)
            vT = jax.lax.dot_general(wvT_ref[w * 128:(w + 1) * 128, :], xn, (((1,), (1,)), ((), ())),
                                     preferred_element_type=jnp.float32)
            vT_sc[w] = jnp.where(onesrow, 1.0, vT).astype(jnp.bfloat16)

        rowq = jax.lax.broadcasted_iota(jnp.int32, (128, MQ), 0)

        def step(t, carry):
            h = t // NQB
            qb = t % NQB
            w = h // 4
            j = h % 4
            kw = k_sc[w]
            q0 = pl.multiple_of(qb * MQ, MQ)
            qTw = qT_sc[w, :, pl.ds(q0, MQ)]
            qm = jnp.where((rowq >= HP * j) & (rowq < HP * j + HP), qTw, jnp.zeros_like(qTw))
            sT = jnp.dot(kw, qm, preferred_element_type=jnp.float32)
            m = jnp.max(sT, axis=0, keepdims=True)
            p = jnp.exp2(sT - m).astype(jnp.bfloat16)
            r0 = pl.multiple_of(j * HP, HP)
            vTh = vT_sc[w, pl.ds(r0, HP), :]
            oT = jnp.dot(vTh, p, preferred_element_type=jnp.float32)
            l = oT[DH:DH + 1, :]
            oT_sc[w, pl.ds(r0, HP), pl.ds(q0, MQ)] = (oT / l).astype(jnp.bfloat16)
            return carry

        jax.lax.fori_loop(0, H * NQB, step, 0)

        oT_all = oT_sc[...].reshape(NW * 128, S)
        attn = jax.lax.dot_general(oT_all, wo_ref[...], (((0,), (0,)), ((), ())),
                                   preferred_element_type=jnp.float32)
        hh = x + attn
        mu2 = jnp.mean(hh, axis=-1, keepdims=True)
        hc = hh - mu2
        var2 = jnp.mean(hc * hc, axis=-1, keepdims=True)
        hn = hc * jax.lax.rsqrt(var2 + 1e-5)
        hnb = hn.astype(jnp.bfloat16).astype(jnp.float32)
        r = jnp.sum(hnb * wr_ref[...].astype(jnp.float32), axis=-1, keepdims=True)
        r = r.astype(jnp.bfloat16).astype(jnp.float32)
        rmax = jnp.max(r, axis=0, keepdims=True)
        ridx = jax.lax.broadcasted_iota(jnp.int32, (S, 1), 0)
        idx = jnp.min(jnp.where(r == rmax, ridx, S), axis=0, keepdims=True)
        sel = ridx == idx
        xsel = jnp.sum(jnp.where(sel, hnb, 0.0), axis=0, keepdims=True)
        xs8 = jnp.broadcast_to(xsel, (8, D)).astype(jnp.bfloat16)
        g = jnp.dot(xs8, wg_ref[...], preferred_element_type=jnp.float32)
        u = jnp.dot(xs8, wu_ref[...], preferred_element_type=jnp.float32)
        gu = (g * jax.nn.sigmoid(g) * u).astype(jnp.bfloat16)
        y = jnp.dot(gu, wd_ref[...], preferred_element_type=jnp.float32)[0:1, :]
        y = y * jax.nn.sigmoid(rmax)
        o_ref[...] = (hh + hn + jnp.where(sel, y, 0.0)).astype(o_ref.dtype)
    return kernel

def build(MQ=256):
    kernel = make_kernel(MQ)
    @jax.jit
    def f(A_x, A_wqkv, A_wo, B_x, B_w_r, B_w_gate, B_w_up, B_w_down):
        x = A_x.reshape(S, D)
        wqkv = A_wqkv.reshape(D, 3, H, DH)
        wqkv = jnp.pad(wqkv, ((0, 0), (0, 0), (0, 0), (0, HP - DH))).reshape(D, 3, H * HP)
        wqT = wqkv[:, 0, :].T
        wk = wqkv[:, 1, :]
        wvT = wqkv[:, 2, :].T
        wo = jnp.pad(A_wo.reshape(H, DH, D), ((0, 0), (0, HP - DH), (0, 0))).reshape(H * HP, D)
        wr = B_w_r.reshape(1, D)
        out = pl.pallas_call(
            kernel,
            out_shape=jax.ShapeDtypeStruct((S, D), jnp.bfloat16),
            scratch_shapes=[pltpu.VMEM((NW, S, 128), jnp.bfloat16),
                            pltpu.VMEM((NW, 128, S), jnp.bfloat16),
                            pltpu.VMEM((NW, 128, S), jnp.bfloat16),
                            pltpu.VMEM((NW, 128, S), jnp.bfloat16)],
            compiler_params=pltpu.CompilerParams(vmem_limit_bytes=100 * 1024 * 1024),
        )(x, wqT, wk, wvT, wo, wr, B_w_gate, B_w_up, B_w_down)
        return out.reshape(1, S, D)
    return f


_IMPL = build()


def pallas_sequential_preLN__mha_block__moe_arch_mod__prompt_kernel(
    A_x, A_wqkv, A_wo, B_x, B_w_r, B_w_gate, B_w_up, B_w_down):
    return _IMPL(A_x, A_wqkv, A_wo, B_x, B_w_r, B_w_gate, B_w_up, B_w_down)
```

```python
import jax
import jax.numpy as jnp
import jax.experimental.pallas as pl
import jax.experimental.pallas.tpu as pltpu

S, D, H, DH, F = 2048, 640, 32, 20, 1536
HP = 32
HPW = 6
NW = 6
LOG2E = 1.4426950408889634

def make_kernel(MQ):
    NQB = S // MQ
    T = H * NQB
    def kernel(x_ref, wqkv_ref, wo_ref, wr_ref, wg_hbm, wu_hbm, wd_hbm, o_ref,
               k_sc, qT_sc, vT_sc, oT_sc, sA, sB, mA, mB, wT_sc, oc_sc, wg_ref, wu_ref, wd_ref, sems):
        cps = [pltpu.make_async_copy(wg_hbm, wg_ref, sems.at[0]),
               pltpu.make_async_copy(wu_hbm, wu_ref, sems.at[1]),
               pltpu.make_async_copy(wd_hbm, wd_ref, sems.at[2])]
        for c in cps:
            c.start()
        wT_sc[...] = wqkv_ref[...].astype(jnp.float32).T

        x = x_ref[...].astype(jnp.float32)
        mu = jnp.mean(x, axis=-1, keepdims=True)
        xc = x - mu
        var = jnp.mean(xc * xc, axis=-1, keepdims=True)
        xn = (xc * jax.lax.rsqrt(var + 1e-5)).astype(jnp.bfloat16)
        scale = (DH ** -0.5) * LOG2E
        nt = (((1,), (1,)), ((), ()))
        for w in range(NW):
            wkT = wT_sc[D + w * 120:D + w * 120 + 128, :].astype(jnp.bfloat16)
            k_sc[w] = jax.lax.dot_general(xn, wkT, nt,
                              preferred_element_type=jnp.float32).astype(jnp.bfloat16)
        qT = jax.lax.dot_general(wT_sc[0:D, :].astype(jnp.bfloat16), xn, nt,
                                 preferred_element_type=jnp.float32)
        qT_sc[0:D, :] = qT * scale
        qT_sc[D:D + 128, :] = jnp.zeros((128, S), jnp.float32)
        vT = jax.lax.dot_general(wT_sc[2 * D:3 * D, :].astype(jnp.bfloat16), xn, nt,
                                 preferred_element_type=jnp.float32)
        rowp = jax.lax.broadcasted_iota(jnp.int32, (HP - DH, S), 0)
        vpad = jnp.where(rowp == 0, 1.0, 0.0)
        for h in range(H):
            vT_sc[h] = jnp.concatenate([vT[DH * h:DH * h + DH, :], vpad], axis=0).astype(jnp.bfloat16)

        rowq = jax.lax.broadcasted_iota(jnp.int32, (128, MQ), 0)

        def stage_a(t, s_ref, m_ref):
            h = t // NQB
            qb = t % NQB
            w = h // HPW
            j = h % HPW
            kw = k_sc[w]
            q0 = pl.multiple_of(qb * MQ, MQ)
            r0 = pl.multiple_of(w * 120, 8)
            qTw = qT_sc[pl.ds(r0, 128), pl.ds(q0, MQ)]
            qm = jnp.where((rowq >= DH * j) & (rowq < DH * j + DH), qTw, 0.0).astype(jnp.bfloat16)
            sT = jnp.dot(kw, qm, preferred_element_type=jnp.float32)
            s_ref[...] = sT
            m_ref[...] = jnp.max(sT, axis=0, keepdims=True)

        def stage_bc(t, s_ref, m_ref):
            h = t // NQB
            qb = t % NQB
            q0 = pl.multiple_of(qb * MQ, MQ)
            p = jnp.exp2(s_ref[...] - m_ref[...]).astype(jnp.bfloat16)
            oT = jnp.dot(vT_sc[h], p, preferred_element_type=jnp.float32)
            l = oT[DH:DH + 1, :]
            oT_sc[h, :, pl.ds(q0, MQ)] = oT / l

        stage_a(0, sA, mA)

        def step(i, carry):
            t0 = 2 * i
            stage_a(t0 + 1, sB, mB)
            stage_bc(t0, sA, mA)
            stage_a(jnp.minimum(t0 + 2, T - 1), sA, mA)
            stage_bc(t0 + 1, sB, mB)
            return carry

        jax.lax.fori_loop(0, T // 2, step, 0)

        for h in range(H):
            oc_sc[DH * h:DH * h + DH, :] = oT_sc[h, 0:DH, :]
        attn = jax.lax.dot_general(oc_sc[...].astype(jnp.bfloat16), wo_ref[...], (((0,), (0,)), ((), ())),
                                   preferred_element_type=jnp.float32)
        hh = x + attn
        mu2 = jnp.mean(hh, axis=-1, keepdims=True)
        hc = hh - mu2
        var2 = jnp.mean(hc * hc, axis=-1, keepdims=True)
        hn = hc * jax.lax.rsqrt(var2 + 1e-5)
        hnb = hn.astype(jnp.bfloat16).astype(jnp.float32)
        r = jnp.sum(hnb * wr_ref[...].astype(jnp.float32), axis=-1, keepdims=True)
        r = r.astype(jnp.bfloat16).astype(jnp.float32)
        rmax = jnp.max(r, axis=0, keepdims=True)
        ridx = jax.lax.broadcasted_iota(jnp.int32, (S, 1), 0)
        idx = jnp.min(jnp.where(r == rmax, ridx, S), axis=0, keepdims=True)
        sel = ridx == idx
        xsel = jnp.sum(jnp.where(sel, hnb, 0.0), axis=0, keepdims=True)
        xs8 = jnp.broadcast_to(xsel, (8, D)).astype(jnp.bfloat16)
        for c in cps:
            c.wait()
        g = jnp.dot(xs8, wg_ref[...], preferred_element_type=jnp.float32)
        u = jnp.dot(xs8, wu_ref[...], preferred_element_type=jnp.float32)
        gu = (g * jax.nn.sigmoid(g) * u).astype(jnp.bfloat16)
        y = jnp.dot(gu, wd_ref[...], preferred_element_type=jnp.float32)[0:1, :]
        y = y * jax.nn.sigmoid(rmax)
        o_ref[...] = (hh + hn + jnp.where(sel, y, 0.0)).astype(o_ref.dtype)
    return kernel

def build(MQ=2048):
    kernel = make_kernel(MQ)
    @jax.jit
    def f(A_x, A_wqkv, A_wo, B_x, B_w_r, B_w_gate, B_w_up, B_w_down):
        x = A_x.reshape(S, D)
        wr = B_w_r.reshape(1, D)
        vm = pl.BlockSpec(memory_space=pltpu.VMEM)
        hb = pl.BlockSpec(memory_space=pl.ANY)
        out = pl.pallas_call(
            kernel,
            out_shape=jax.ShapeDtypeStruct((S, D), jnp.bfloat16),
            in_specs=[vm, vm, vm, vm, hb, hb, hb],
            scratch_shapes=[pltpu.VMEM((NW, S, 128), jnp.bfloat16),
                            pltpu.VMEM((D + 128, S), jnp.float32),
                            pltpu.VMEM((H, HP, S), jnp.bfloat16),
                            pltpu.VMEM((H, HP, S), jnp.float32),
                            pltpu.VMEM((S, MQ), jnp.float32),
                            pltpu.VMEM((S, MQ), jnp.float32),
                            pltpu.VMEM((1, MQ), jnp.float32),
                            pltpu.VMEM((1, MQ), jnp.float32),
                            pltpu.VMEM((3 * D, D), jnp.float32),
                            pltpu.VMEM((D, S), jnp.float32),
                            pltpu.VMEM((D, F), jnp.bfloat16),
                            pltpu.VMEM((D, F), jnp.bfloat16),
                            pltpu.VMEM((F, D), jnp.bfloat16),
                            pltpu.SemaphoreType.DMA((3,))],
            compiler_params=pltpu.CompilerParams(vmem_limit_bytes=120 * 1024 * 1024),
        )(x, A_wqkv, A_wo, wr, B_w_gate, B_w_up, B_w_down)
        return out.reshape(1, S, D)
    return f


_IMPL = build()


def pallas_sequential_preLN__mha_block__moe_arch_mod__prompt_kernel(
    A_x, A_wqkv, A_wo, B_x, B_w_r, B_w_gate, B_w_up, B_w_down):
    return _IMPL(A_x, A_wqkv, A_wo, B_x, B_w_r, B_w_gate, B_w_up, B_w_down)
```

```python
import jax
import jax.numpy as jnp
import jax.experimental.pallas as pl
import jax.experimental.pallas.tpu as pltpu

S, D, H, DH, F = 2048, 640, 32, 20, 1536
HP = 32
HPW = 6
NW = 6
LOG2E = 1.4426950408889634

def make_kernel(MQ):
    NQB = S // MQ
    T = H * NQB
    def kernel(x_ref, wqkv_ref, wo_ref, wr_ref, wg_hbm, wu_hbm, wd_hbm, o_ref,
               k_sc, qT_sc, vT_sc, oT_sc, sA, sB, mA, mB, wT_sc, oc_sc, wg_ref, wu_ref, wd_ref, sems):
        cps = [pltpu.make_async_copy(wg_hbm, wg_ref, sems.at[0]),
               pltpu.make_async_copy(wu_hbm, wu_ref, sems.at[1]),
               pltpu.make_async_copy(wd_hbm, wd_ref, sems.at[2])]
        for c in cps:
            c.start()
        wT_sc[...] = wqkv_ref[...].astype(jnp.float32).T

        x = x_ref[...].astype(jnp.float32)
        mu = jnp.mean(x, axis=-1, keepdims=True)
        xc = x - mu
        var = jnp.mean(xc * xc, axis=-1, keepdims=True)
        xn = (xc * jax.lax.rsqrt(var + 1e-5)).astype(jnp.bfloat16)
        scale = (DH ** -0.5) * LOG2E
        nt = (((1,), (1,)), ((), ()))
        for w in range(NW):
            wkT = wT_sc[D + w * 120:D + w * 120 + 128, :].astype(jnp.bfloat16)
            k_sc[w] = jax.lax.dot_general(xn, wkT, nt,
                              preferred_element_type=jnp.float32).astype(jnp.bfloat16)
        qT = jax.lax.dot_general(wT_sc[0:D, :].astype(jnp.bfloat16), xn, nt,
                                 preferred_element_type=jnp.float32)
        qT_sc[0:D, :] = qT * scale
        qT_sc[D:D + 128, :] = jnp.zeros((128, S), jnp.float32)
        vT = jax.lax.dot_general(wT_sc[2 * D:3 * D, :].astype(jnp.bfloat16), xn, nt,
                                 preferred_element_type=jnp.float32)
        rowp = jax.lax.broadcasted_iota(jnp.int32, (HP - DH, S), 0)
        vpad = jnp.where(rowp == 0, 1.0, 0.0)
        for h in range(H):
            vT_sc[h] = jnp.concatenate([vT[DH * h:DH * h + DH, :], vpad], axis=0).astype(jnp.bfloat16)

        rowq = jax.lax.broadcasted_iota(jnp.int32, (128, MQ), 0)

        def stage_a(t, s_ref, m_ref):
            h = t // NQB
            qb = t % NQB
            w = h // HPW
            j = h % HPW
            kw = k_sc[w]
            q0 = pl.multiple_of(qb * MQ, MQ)
            r0 = pl.multiple_of(w * 120, 8)
            qTw = qT_sc[pl.ds(r0, 128), pl.ds(q0, MQ)]
            qm = jnp.where((rowq >= DH * j) & (rowq < DH * j + DH), qTw, 0.0).astype(jnp.bfloat16)
            sT = jnp.dot(kw, qm, preferred_element_type=jnp.float32)
            s_ref[...] = sT
            m_ref[...] = jnp.max(sT, axis=0, keepdims=True)

        def stage_bc(t, s_ref, m_ref):
            h = t // NQB
            qb = t % NQB
            q0 = pl.multiple_of(qb * MQ, MQ)
            p = jnp.exp2(s_ref[...] - m_ref[...]).astype(jnp.bfloat16)
            oT = jnp.dot(vT_sc[h], p, preferred_element_type=jnp.float32)
            l = oT[DH:DH + 1, :]
            oT_sc[h, :, pl.ds(q0, MQ)] = oT / l

        stage_a(0, sA, mA)

        def step(i, carry):
            t0 = 2 * i
            stage_a(t0 + 1, sB, mB)
            stage_bc(t0, sA, mA)
            stage_a(t0 + 2, sA, mA)
            stage_bc(t0 + 1, sB, mB)
            return carry

        jax.lax.fori_loop(0, T // 2 - 1, step, 0)
        stage_a(T - 1, sB, mB)
        stage_bc(T - 2, sA, mA)
        stage_bc(T - 1, sB, mB)

        for h in range(H):
            oc_sc[DH * h:DH * h + DH, :] = oT_sc[h, 0:DH, :]
        attn = jax.lax.dot_general(oc_sc[...].astype(jnp.bfloat16), wo_ref[...], (((0,), (0,)), ((), ())),
                                   preferred_element_type=jnp.float32)
        hh = x + attn
        mu2 = jnp.mean(hh, axis=-1, keepdims=True)
        hc = hh - mu2
        var2 = jnp.mean(hc * hc, axis=-1, keepdims=True)
        hn = hc * jax.lax.rsqrt(var2 + 1e-5)
        hnb = hn.astype(jnp.bfloat16).astype(jnp.float32)
        r = jnp.sum(hnb * wr_ref[...].astype(jnp.float32), axis=-1, keepdims=True)
        r = r.astype(jnp.bfloat16).astype(jnp.float32)
        rmax = jnp.max(r, axis=0, keepdims=True)
        ridx = jax.lax.broadcasted_iota(jnp.int32, (S, 1), 0)
        idx = jnp.min(jnp.where(r == rmax, ridx, S), axis=0, keepdims=True)
        sel = ridx == idx
        xsel = jnp.sum(jnp.where(sel, hnb, 0.0), axis=0, keepdims=True)
        xs8 = jnp.broadcast_to(xsel, (8, D)).astype(jnp.bfloat16)
        for c in cps:
            c.wait()
        g = jnp.dot(xs8, wg_ref[...], preferred_element_type=jnp.float32)
        u = jnp.dot(xs8, wu_ref[...], preferred_element_type=jnp.float32)
        gu = (g * jax.nn.sigmoid(g) * u).astype(jnp.bfloat16)
        y = jnp.dot(gu, wd_ref[...], preferred_element_type=jnp.float32)[0:1, :]
        y = y * jax.nn.sigmoid(rmax)
        o_ref[...] = (hh + hn + jnp.where(sel, y, 0.0)).astype(o_ref.dtype)
    return kernel

def build(MQ=2048):
    kernel = make_kernel(MQ)
    @jax.jit
    def f(A_x, A_wqkv, A_wo, B_x, B_w_r, B_w_gate, B_w_up, B_w_down):
        x = A_x.reshape(S, D)
        wr = B_w_r.reshape(1, D)
        vm = pl.BlockSpec(memory_space=pltpu.VMEM)
        hb = pl.BlockSpec(memory_space=pl.ANY)
        out = pl.pallas_call(
            kernel,
            out_shape=jax.ShapeDtypeStruct((S, D), jnp.bfloat16),
            in_specs=[vm, vm, vm, vm, hb, hb, hb],
            scratch_shapes=[pltpu.VMEM((NW, S, 128), jnp.bfloat16),
                            pltpu.VMEM((D + 128, S), jnp.float32),
                            pltpu.VMEM((H, HP, S), jnp.bfloat16),
                            pltpu.VMEM((H, HP, S), jnp.float32),
                            pltpu.VMEM((S, MQ), jnp.float32),
                            pltpu.VMEM((S, MQ), jnp.float32),
                            pltpu.VMEM((1, MQ), jnp.float32),
                            pltpu.VMEM((1, MQ), jnp.float32),
                            pltpu.VMEM((3 * D, D), jnp.float32),
                            pltpu.VMEM((D, S), jnp.float32),
                            pltpu.VMEM((D, F), jnp.bfloat16),
                            pltpu.VMEM((D, F), jnp.bfloat16),
                            pltpu.VMEM((F, D), jnp.bfloat16),
                            pltpu.SemaphoreType.DMA((3,))],
            compiler_params=pltpu.CompilerParams(vmem_limit_bytes=120 * 1024 * 1024),
        )(x, A_wqkv, A_wo, wr, B_w_gate, B_w_up, B_w_down)
        return out.reshape(1, S, D)
    return f


_IMPL = build()


def pallas_sequential_preLN__mha_block__moe_arch_mod__prompt_kernel(
    A_x, A_wqkv, A_wo, B_x, B_w_r, B_w_gate, B_w_up, B_w_down):
    return _IMPL(A_x, A_wqkv, A_wo, B_x, B_w_r, B_w_gate, B_w_up, B_w_down)
```
